```python
import jax
import jax.numpy as jnp

def _softmax(x, axis=-1):
    return jax.nn.softmax(x, axis=axis)
def _gelu(x):
    return jax.nn.gelu(x, approximate=True)
def _silu(x):
    return jax.nn.silu(x)
def _sigmoid(x):
    return jax.nn.sigmoid(x)
def _layernorm(x, axis=-1, eps=1e-5):
    m = jnp.mean(x, axis=axis, keepdims=True)
    v = jnp.var(x, axis=axis, keepdims=True)
    return (x - m) / jnp.sqrt(v + eps)
def _scatter_add(tgt, idx, src, axis=0):
    return tgt.at[idx].add(src)
def _segment_sum(src, seg, n):
    return jax.ops.segment_sum(src, seg, n)
class _Rng:
    def __init__(self, key):
        self._k = key
    def _next(self):
        self._k, sub = jax.random.split(self._k)
        return sub
    def normal(self, shape):
        return jax.random.normal(self._next(), shape, dtype=jnp.bfloat16)
    def randint(self, lo, hi, shape):
        return jax.random.randint(self._next(), shape, lo, hi, dtype=jnp.int32)
    def uniform(self, shape, lo=0.0, hi=1.0):
        return jax.random.uniform(self._next(), shape, jnp.bfloat16, lo, hi)
    def permutation(self, n):
        return jax.random.permutation(self._next(), n)


kernel_name = 'gated_mix__sliding_block_cached__dense_activation_gelu__decode'

def setup_inputs():
    _rng = _Rng(jax.random.key(int.from_bytes(__import__("os").urandom(4), "little")))
    _w = (lambda a: (lambda t: t.astype(jnp.bfloat16) if jnp.issubdtype(t.dtype, jnp.floating) else t)(jnp.asarray(a)))
    def _A_setup():
        B, Sq, D = 1, 1, 640
        Hq, Hkv, Sk, Dh = 32, 32, 32768, 192
        assert Hq % Hkv == 0, (Hq, Hkv)
        return {
            "x": _w((lambda *s: _rng.normal(s) * 0.05)(B, Sq, D)),
            "k_cache": _w((lambda *s: _rng.normal(s) * 0.05)(B, Hkv, Sk, Dh)),
            "v_cache": _w((lambda *s: _rng.normal(s) * 0.05)(B, Hkv, Sk, Dh)),
            "wq": _w((lambda *s: _rng.normal(s) * 0.05)(D, Hq * Dh) * (D ** -0.5)),
            "wo": _w((lambda *s: _rng.normal(s) * 0.05)(Hq * Dh, D) * ((Hq * Dh) ** -0.5)),
        }
    _A_in = _A_setup()

    def _B_setup():
        B, S, D, F = 1, 1, 640, 1536
        return {
            "x": _w((lambda *s: _rng.normal(s) * 0.05)(B, S, D)),
            "w1": _w((lambda *s: _rng.normal(s) * 0.05)(D, F) * (D ** -0.5)),
            "b1": _w((lambda *s: _rng.normal(s) * 0.05)(F) * 0.01),
            "w2": _w((lambda *s: _rng.normal(s) * 0.05)(F, D) * (F ** -0.5)),
            "b2": _w((lambda *s: _rng.normal(s) * 0.05)(D) * 0.01),
        }
    _B_in = _B_setup()

    return {
        "A_x": _A_in["x"],
        "A_k_cache": _A_in["k_cache"],
        "A_v_cache": _A_in["v_cache"],
        "A_wq": _A_in["wq"],
        "A_wo": _A_in["wo"],
        "B_x": _B_in["x"],
        "B_w1": _B_in["w1"],
        "B_b1": _B_in["b1"],
        "B_w2": _B_in["w2"],
        "B_b2": _B_in["b2"],
        "gate_w": _w((lambda *s: _rng.normal(s) * 0.05)(640)),
    }

def reference(A_x, A_k_cache, A_v_cache, A_wq, A_wo, B_x, B_w1, B_b1, B_w2, B_b2, gate_w):
    def _A_ref(x, k_cache, v_cache, wq, wo):
        B, Sq, D = x.shape
        Hq, Dh = 32, 192
        Hkv, Sk = k_cache.shape[1], k_cache.shape[2]
        W = min(4096, max(256, Sk // 4))
        rep = Hq // Hkv
        q = (lambda x, *d: x.transpose(*d))((x @ wq).reshape(B, Sq, Hq, Dh), 0, 2, 1, 3)
        k = jnp.repeat(k_cache[:, :, Sk - W:, :], rep, axis=1)
        v = jnp.repeat(v_cache[:, :, Sk - W:, :], rep, axis=1)
        scores = jnp.einsum("bhqd,bhkd->bhqk", q, k) * (Dh ** -0.5)
        p = _softmax(scores, axis=-1)
        o = jnp.einsum("bhqk,bhkd->bhqd", p, v)
        return (lambda x, *d: x.transpose(*d))(o, 0, 2, 1, 3).reshape(B, Sq, Hq * Dh) @ wo

    def _B_ref(x, w1, b1, w2, b2):
        h = jnp.einsum("bsd,df->bsf", x, w1) + b1
        h = _gelu(h)
        return jnp.einsum("bsf,fd->bsd", h, w2) + b2

    x = A_x
    g = _sigmoid((x * gate_w).sum(-1, keepdims=True))
    a = _A_ref(x, A_k_cache, A_v_cache, A_wq, A_wo)
    b = _B_ref(x, B_w1, B_b1, B_w2, B_b2)
    return g * a + (1 - g) * b
```

```python
import functools

import jax
import jax.numpy as jnp
import jax.experimental.pallas as pl
import jax.experimental.pallas.tpu as pltpu

_HEADS_PER_GROUP = 2
_ROWS = 8
_NBUF = 2
_WO_SLICES = 8


def _kernel(x_hbm, gw_hbm, b1_hbm, b2_hbm, k_hbm, v_hbm, wq_hbm, wo_hbm, w1_hbm, w2_hbm,
            o_ref,
            x_v, gw_v, b1_v, b2_v, kbuf, vbuf, wq_v, wo_v, w1_v, w2_v, o_scr,
            ksem, vsem, wsem, ssem, wosem,
            *, head_dim):
    f32, bf16 = jnp.float32, jnp.bfloat16
    nbuf, gd, win = kbuf.shape
    d_model = o_ref.shape[-1]
    d_ff = w1_v.shape[1]
    seq = k_hbm.shape[1]
    n_groups = k_hbm.shape[0] // gd
    n_wo = wosem.shape[0]
    wo_rows = wo_v.shape[0] // n_wo
    wo_per_step = n_wo // (2 * nbuf)

    def kv_copy(src, buf, sem, g, slot):
        rows = pl.ds(pl.multiple_of(g * gd, gd), gd)
        return pltpu.make_async_copy(src.at[rows, pl.ds(seq - win, win)], buf.at[slot], sem.at[slot])

    k_copy = functools.partial(kv_copy, k_hbm, kbuf, ksem)
    v_copy = functools.partial(kv_copy, v_hbm, vbuf, vsem)

    def wo_copy(j):
        rows = pl.ds(pl.multiple_of(j * wo_rows, wo_rows), wo_rows)
        return pltpu.make_async_copy(wo_hbm.at[rows, :], wo_v.at[rows, :], wosem.at[j])

    wq_copy = pltpu.make_async_copy(wq_hbm, wq_v, wsem.at[0])
    w1_copy = pltpu.make_async_copy(w1_hbm, w1_v, wsem.at[1])
    w2_copy = pltpu.make_async_copy(w2_hbm, w2_v, wsem.at[2])
    small_copies = [
        pltpu.make_async_copy(src, dst, ssem.at[i])
        for i, (src, dst) in enumerate(((x_hbm, x_v), (gw_hbm, gw_v), (b1_hbm, b1_v), (b2_hbm, b2_v)))
    ]

    wq_copy.start()
    for c in small_copies:
        c.start()
    w1_copy.start()
    w2_copy.start()
    for g in range(nbuf):
        k_copy(g, g).start()
        v_copy(g, g).start()

    for c in small_copies:
        c.wait()
    x = x_v[...]
    x_rows = jnp.broadcast_to(x, (_ROWS, d_model))
    gate = jax.nn.sigmoid(
        jnp.sum(x.astype(f32) * gw_v[...].astype(f32).reshape(1, d_model), axis=-1, keepdims=True))
    w1_copy.wait()
    h = jnp.dot(x_rows, w1_v[...], preferred_element_type=f32) + b1_v[...].astype(f32).reshape(1, d_ff)
    h = jax.nn.gelu(h.astype(bf16).astype(f32), approximate=True)
    w2_copy.wait()
    ffn = jnp.dot(h.astype(bf16), w2_v[...], preferred_element_type=f32)
    ffn = ffn + b2_v[...].astype(f32).reshape(1, d_model)

    row = jax.lax.broadcasted_iota(jnp.int32, (_ROWS, gd), 0)
    col = jax.lax.broadcasted_iota(jnp.int32, (_ROWS, gd), 1)
    own = (col >= row * head_dim) & (col < (row + 1) * head_dim)
    wq_copy.wait()

    def step(g, carry):
        slot = g % nbuf
        cols = pl.ds(pl.multiple_of(g * gd, 128), gd)
        more_kv = g + nbuf < n_groups
        wo_base = (g + nbuf - n_groups) * 2 * wo_per_step

        q = jnp.dot(x_rows, wq_v[:, cols], preferred_element_type=f32)
        q_bd = jnp.where(own, q, 0.0).astype(bf16)

        k_copy(g, slot).wait()
        s = jnp.dot(q_bd, kbuf[slot], preferred_element_type=f32) * (head_dim ** -0.5)

        @pl.when(more_kv)
        def _():
            k_copy(g + nbuf, slot).start()

        @pl.when(jnp.logical_not(more_kv))
        def _():
            for t in range(wo_per_step):
                wo_copy(wo_base + t).start()

        m = jnp.max(s, axis=-1, keepdims=True)
        e = jnp.exp(s - m)
        p = (e / jnp.sum(e, axis=-1, keepdims=True)).astype(bf16)

        v_copy(g, slot).wait()
        o = jax.lax.dot_general(p, vbuf[slot], (((1,), (1,)), ((), ())), preferred_element_type=f32)

        @pl.when(more_kv)
        def _():
            v_copy(g + nbuf, slot).start()

        @pl.when(jnp.logical_not(more_kv))
        def _():
            for t in range(wo_per_step):
                wo_copy(wo_base + wo_per_step + t).start()

        o_scr[:, cols] = jnp.where(own, o, 0.0).astype(bf16)
        return carry

    jax.lax.fori_loop(0, n_groups, step, 0)

    acc = jnp.zeros((_ROWS, d_model), f32)
    for j in range(n_wo):
        rows = slice(j * wo_rows, (j + 1) * wo_rows)
        wo_copy(j).wait()
        acc = acc + jnp.dot(o_scr[:, rows], wo_v[rows, :], preferred_element_type=f32)
    attn = jnp.sum(acc, axis=0, keepdims=True)
    o_ref[...] = (gate * attn + (1.0 - gate) * ffn[0:1]).astype(o_ref.dtype)


@jax.jit
def pallas_gated_mix__sliding_block_cached__dense_activation_gelu__decode_kernel(
    A_x: jax.Array,
    A_k_cache: jax.Array,
    A_v_cache: jax.Array,
    A_wq: jax.Array,
    A_wo: jax.Array,
    B_x: jax.Array,
    B_w1: jax.Array,
    B_b1: jax.Array,
    B_w2: jax.Array,
    B_b2: jax.Array,
    gate_w: jax.Array,
):
    del B_x
    batch, sq, d_model = A_x.shape
    _, n_heads, seq, head_dim = A_k_cache.shape
    d_ff = B_w1.shape[1]
    win = min(4096, max(256, seq // 4))
    gd = _HEADS_PER_GROUP * head_dim
    assert batch * sq == 1 and A_wq.shape == (d_model, n_heads * head_dim)
    assert n_heads % _HEADS_PER_GROUP == 0 and gd % 128 == 0 and win % 128 == 0 and (seq - win) % 128 == 0
    assert _WO_SLICES % (2 * _NBUF) == 0 and (n_heads * head_dim) % (128 * _WO_SLICES) == 0

    k_t = jnp.swapaxes(A_k_cache, 2, 3).reshape(n_heads * head_dim, seq)
    v_t = jnp.swapaxes(A_v_cache, 2, 3).reshape(n_heads * head_dim, seq)

    bf16 = jnp.bfloat16
    hbm = pl.BlockSpec(memory_space=pl.ANY)
    out = pl.pallas_call(
        functools.partial(_kernel, head_dim=head_dim),
        in_specs=[hbm] * 10,
        out_specs=pl.BlockSpec(memory_space=pltpu.VMEM),
        out_shape=jax.ShapeDtypeStruct((1, d_model), A_x.dtype),
        scratch_shapes=[
            pltpu.VMEM((1, d_model), bf16),
            pltpu.VMEM((d_model,), bf16),
            pltpu.VMEM((d_ff,), bf16),
            pltpu.VMEM((d_model,), bf16),
            pltpu.VMEM((_NBUF, gd, win), bf16),
            pltpu.VMEM((_NBUF, gd, win), bf16),
            pltpu.VMEM(A_wq.shape, bf16),
            pltpu.VMEM(A_wo.shape, bf16),
            pltpu.VMEM(B_w1.shape, bf16),
            pltpu.VMEM(B_w2.shape, bf16),
            pltpu.VMEM((_ROWS, n_heads * head_dim), bf16),
            pltpu.SemaphoreType.DMA((_NBUF,)),
            pltpu.SemaphoreType.DMA((_NBUF,)),
            pltpu.SemaphoreType.DMA((3,)),
            pltpu.SemaphoreType.DMA((4,)),
            pltpu.SemaphoreType.DMA((_WO_SLICES,)),
        ],
        compiler_params=pltpu.CompilerParams(vmem_limit_bytes=64 * 1024 * 1024),
    )(A_x.reshape(1, d_model), gate_w, B_b1, B_b2, k_t, v_t, A_wq, A_wo, B_w1, B_w2)
    return out.reshape(batch, sq, d_model)
```

```python
import functools

import jax
import jax.numpy as jnp
from jax import lax
import jax.experimental.pallas as pl
import jax.experimental.pallas.tpu as pltpu

_HEADS_PER_GROUP = 2
_ROWS = 8
_NBUF = 2
_WO_SLICES = 8
_KV_CHUNK = 1024
_FF_CHUNK = 256
_LANE = 128


def _kernel(x_hbm, gw_hbm, b1_hbm, b2_hbm, k_hbm, v_hbm, wq_hbm, wo_hbm, w1_hbm, w2_hbm,
            o_ref,
            x_v, gw_v, b1_v, b2_v, kbuf, vbuf, wq_v, wo_v, w1_v, w2_v, o_scr, s_scr, p_scr, b1_f,
            ksem, vsem, wsem, ssem, wosem,
            *, head_dim):
    f32, bf16 = jnp.float32, jnp.bfloat16
    aligned = pl.multiple_of
    nbuf, gd, win = kbuf.shape
    d_model = o_ref.shape[-1]
    d_ff = w1_v.shape[1]
    seq = k_hbm.shape[1]
    n_groups = k_hbm.shape[0] // gd
    n_wo = wosem.shape[0]
    wo_rows = wo_v.shape[0] // n_wo
    wo_per_step = n_wo // (2 * nbuf)

    def kv_start(src, buf, sem, g, slot):
        def issue(c, carry):
            col = aligned(c * _LANE, _LANE)
            for r in range(_HEADS_PER_GROUP):
                pltpu.make_async_copy(
                    src.at[pl.ds(aligned(g * gd + r * head_dim, 8), head_dim), pl.ds(seq - win + col, _LANE)],
                    buf.at[slot, pl.ds(r * head_dim, head_dim), pl.ds(col, _LANE)],
                    sem.at[slot],
                ).start(priority=r)
            return carry

        lax.fori_loop(0, win // _LANE, issue, 0)

    def kv_wait(buf, sem, slot):
        pltpu.make_async_copy(buf.at[slot], buf.at[slot], sem.at[slot]).wait()

    def rows_start(src, dst, sem, row0, nrows, piece_rows, piece_cols=None):
        cols = src.shape[1]
        piece_cols = cols if piece_cols is None else piece_cols
        ncol = cols // piece_cols
        per_queue = (nrows // piece_rows) * ncol // 2

        def issue(i, carry):
            for queue in range(2):
                j = i + queue * per_queue
                r = pl.ds(aligned(row0 + (j // ncol) * piece_rows, 8), piece_rows)
                c = pl.ds(aligned((j % ncol) * piece_cols, _LANE), piece_cols)
                pltpu.make_async_copy(src.at[r, c], dst.at[r, c], sem).start(priority=queue)
            return carry

        lax.fori_loop(0, per_queue, issue, 0)

    def full_wait(dst, sem):
        pltpu.make_async_copy(dst, dst, sem).wait()

    def wo_start(j):
        rows_start(wo_hbm, wo_v, wosem.at[j], j * wo_rows, wo_rows, 32)

    def wo_wait(j):
        full_wait(wo_v.at[pl.ds(aligned(j * wo_rows, 8), wo_rows)], wosem.at[j])

    small_copies = [
        pltpu.make_async_copy(src, dst, ssem.at[i])
        for i, (src, dst) in enumerate(((x_hbm, x_v), (gw_hbm, gw_v), (b1_hbm, b1_v), (b2_hbm, b2_v)))
    ]

    rows_start(wq_hbm, wq_v, wsem.at[0], 0, d_model, 8, wq_v.shape[1] // 2)
    for c in small_copies:
        c.start()
    rows_start(w1_hbm, w1_v, wsem.at[1], 0, d_model, 8)
    rows_start(w2_hbm, w2_v, wsem.at[2], 0, d_ff, 32)
    for g in range(nbuf):
        kv_start(k_hbm, kbuf, ksem, g, g)
        kv_start(v_hbm, vbuf, vsem, g, g)

    for c in small_copies:
        c.wait()
    x = x_v[...]
    x_rows = jnp.broadcast_to(x, (_ROWS, d_model))
    gate = jax.nn.sigmoid(
        jnp.sum(x.astype(f32) * gw_v[...].astype(f32).reshape(1, d_model), axis=-1, keepdims=True))
    b1_f[...] = jnp.broadcast_to(b1_v[...].astype(f32).reshape(1, d_ff), (_ROWS, d_ff))
    full_wait(w1_v, wsem.at[1])
    full_wait(w2_v, wsem.at[2])

    def ffn_step(j, acc):
        cs = pl.ds(aligned(j * _FF_CHUNK, _LANE), _FF_CHUNK)
        h = jnp.dot(x_rows, w1_v[:, cs], preferred_element_type=f32) + b1_f[:, cs]
        h = jax.nn.gelu(h.astype(bf16).astype(f32), approximate=True).astype(bf16)
        return acc + jnp.dot(h, w2_v[cs, :], preferred_element_type=f32)

    ffn = lax.fori_loop(0, d_ff // _FF_CHUNK, ffn_step, jnp.zeros((_ROWS, d_model), f32))
    ffn = ffn + b2_v[...].astype(f32).reshape(1, d_model)

    full_wait(wq_v, wsem.at[0])
    row = lax.broadcasted_iota(jnp.int32, (_ROWS, gd), 0)
    col = lax.broadcasted_iota(jnp.int32, (_ROWS, gd), 1)
    own = (col >= row * head_dim) & (col < (row + 1) * head_dim)

    def group_step(g, carry):
        slot = g % nbuf
        cols = pl.ds(aligned(g * gd, _LANE), gd)
        more_kv = g + nbuf < n_groups
        wo_base = (g + nbuf - n_groups) * 2 * wo_per_step

        q = jnp.dot(x_rows, wq_v[:, cols], preferred_element_type=f32)
        q_bd = jnp.where(own, q, 0.0).astype(bf16)

        kv_wait(kbuf, ksem, slot)

        def qk_step(c, m):
            cs = pl.ds(aligned(c * _KV_CHUNK, _LANE), _KV_CHUNK)
            s = jnp.dot(q_bd, kbuf[slot, :, cs], preferred_element_type=f32) * (head_dim ** -0.5)
            s_scr[:, cs] = s
            return jnp.maximum(m, jnp.max(s, axis=-1, keepdims=True))

        m = lax.fori_loop(0, win // _KV_CHUNK, qk_step, jnp.full((_ROWS, 1), -jnp.inf, f32))

        @pl.when(more_kv)
        def _():
            kv_start(k_hbm, kbuf, ksem, g + nbuf, slot)

        @pl.when(jnp.logical_not(more_kv))
        def _():
            for t in range(wo_per_step):
                wo_start(wo_base + t)

        e = jnp.exp(s_scr[...] - m)
        p_scr[...] = (e / jnp.sum(e, axis=-1, keepdims=True)).astype(bf16)

        kv_wait(vbuf, vsem, slot)

        def pv_step(c, o):
            cs = pl.ds(aligned(c * _KV_CHUNK, _LANE), _KV_CHUNK)
            return o + lax.dot_general(p_scr[:, cs], vbuf[slot, :, cs], (((1,), (1,)), ((), ())),
                                       preferred_element_type=f32)

        o = lax.fori_loop(0, win // _KV_CHUNK, pv_step, jnp.zeros((_ROWS, gd), f32))

        @pl.when(more_kv)
        def _():
            kv_start(v_hbm, vbuf, vsem, g + nbuf, slot)

        @pl.when(jnp.logical_not(more_kv))
        def _():
            for t in range(wo_per_step):
                wo_start(wo_base + wo_per_step + t)

        o_scr[:, cols] = jnp.where(own, o, 0.0).astype(bf16)
        return carry

    lax.fori_loop(0, n_groups, group_step, 0)

    def wo_step(j, acc):
        wo_wait(j)
        rs = pl.ds(aligned(j * wo_rows, _LANE), wo_rows)
        return acc + jnp.dot(o_scr[:, rs], wo_v[rs, :], preferred_element_type=f32)

    acc = lax.fori_loop(0, n_wo, wo_step, jnp.zeros((_ROWS, d_model), f32))
    attn = jnp.sum(acc, axis=0, keepdims=True)
    o_ref[...] = (gate * attn + (1.0 - gate) * ffn[0:1]).astype(o_ref.dtype)


@jax.jit
def pallas_gated_mix__sliding_block_cached__dense_activation_gelu__decode_kernel(
    A_x: jax.Array,
    A_k_cache: jax.Array,
    A_v_cache: jax.Array,
    A_wq: jax.Array,
    A_wo: jax.Array,
    B_x: jax.Array,
    B_w1: jax.Array,
    B_b1: jax.Array,
    B_w2: jax.Array,
    B_b2: jax.Array,
    gate_w: jax.Array,
):
    del B_x
    batch, sq, d_model = A_x.shape
    _, n_heads, seq, head_dim = A_k_cache.shape
    d_ff = B_w1.shape[1]
    win = min(4096, max(256, seq // 4))
    gd = _HEADS_PER_GROUP * head_dim
    d_attn = n_heads * head_dim
    assert batch * sq == 1 and A_wq.shape == (d_model, d_attn) and A_wo.shape == (d_attn, d_model)
    assert n_heads % _HEADS_PER_GROUP == 0 and gd % _LANE == 0 and head_dim % 8 == 0
    assert win % _KV_CHUNK == 0 and (seq - win) % _LANE == 0 and d_ff % _FF_CHUNK == 0
    assert _WO_SLICES % (2 * _NBUF) == 0 and d_attn % (_LANE * _WO_SLICES) == 0
    assert d_model % 16 == 0 and d_ff % 64 == 0 and d_attn % 256 == 0

    k_t = jnp.swapaxes(A_k_cache, 2, 3).reshape(d_attn, seq)
    v_t = jnp.swapaxes(A_v_cache, 2, 3).reshape(d_attn, seq)

    bf16, f32 = jnp.bfloat16, jnp.float32
    hbm = pl.BlockSpec(memory_space=pl.ANY)
    out = pl.pallas_call(
        functools.partial(_kernel, head_dim=head_dim),
        in_specs=[hbm] * 10,
        out_specs=pl.BlockSpec(memory_space=pltpu.VMEM),
        out_shape=jax.ShapeDtypeStruct((1, d_model), A_x.dtype),
        scratch_shapes=[
            pltpu.VMEM((1, d_model), bf16),
            pltpu.VMEM((d_model,), bf16),
            pltpu.VMEM((d_ff,), bf16),
            pltpu.VMEM((d_model,), bf16),
            pltpu.VMEM((_NBUF, gd, win), bf16),
            pltpu.VMEM((_NBUF, gd, win), bf16),
            pltpu.VMEM(A_wq.shape, bf16),
            pltpu.VMEM(A_wo.shape, bf16),
            pltpu.VMEM(B_w1.shape, bf16),
            pltpu.VMEM(B_w2.shape, bf16),
            pltpu.VMEM((_ROWS, d_attn), bf16),
            pltpu.VMEM((_ROWS, win), f32),
            pltpu.VMEM((_ROWS, win), bf16),
            pltpu.VMEM((_ROWS, d_ff), f32),
            pltpu.SemaphoreType.DMA((_NBUF,)),
            pltpu.SemaphoreType.DMA((_NBUF,)),
            pltpu.SemaphoreType.DMA((3,)),
            pltpu.SemaphoreType.DMA((4,)),
            pltpu.SemaphoreType.DMA((_WO_SLICES,)),
        ],
        compiler_params=pltpu.CompilerParams(vmem_limit_bytes=64 * 1024 * 1024),
    )(A_x.reshape(1, d_model), gate_w, B_b1, B_b2, k_t, v_t, A_wq, A_wo, B_w1, B_w2)
    return out.reshape(batch, sq, d_model)
```

```python
import functools

import jax
import jax.numpy as jnp
from jax import lax
import jax.experimental.pallas as pl
import jax.experimental.pallas.tpu as pltpu

_LANE = 128
_ROWS = 8
_HEADS_PER_GROUP = 2
_AHEAD = 2
_NBUF = _AHEAD + 1
_KV_CHUNKS = 2
_FF_CHUNK = 256
_WO_SEGS = 8
_WO_CHUNK = _LANE
_WO_PIECE = 32
_WO_LAST_PARTS = 4


def _log2(n):
    assert n & (n - 1) == 0, n
    return n.bit_length() - 1


def _kernel(x_hbm, gw_hbm, b1_hbm, b2_hbm, k_hbm, v_hbm, wq_hbm, wo_hbm, w1_hbm, w2_hbm,
            o_ref,
            x_v, gw_v, b1_v, b2_v, kbuf, vbuf, wq_v, wo_v, w1_v, w2_v, o_scr, s_scr, p_scr, b1_f,
            ksem, vsem, wsem, ssem, wosem,
            *, head_dim):
    f32, bf16 = jnp.float32, jnp.bfloat16
    aligned = pl.multiple_of
    _, gd, win = kbuf.shape
    d_model = o_ref.shape[-1]
    d_ff = w1_v.shape[1]
    seq = k_hbm.shape[1]
    n_groups = k_hbm.shape[0] // gd
    kv_cols = win // _KV_CHUNKS
    kv_tiles = gd // 8
    steps = 2 * _KV_CHUNKS
    n_slices = wo_v.shape[0]
    last = n_slices - 1
    seg_rows = wo_hbm.shape[0] // _WO_SEGS
    seg_pairs = _WO_SEGS // 2
    per_chunk = _WO_CHUNK // _WO_PIECE
    pairs_per_slice = seg_pairs * per_chunk

    def kv_issue(g, slot, step):
        col = aligned((step >> 1) * kv_cols, _LANE)

        def issue(i, carry):
            row = aligned((2 * i + (step & 1)) * 8, 8)
            for queue, (src, buf, sem) in enumerate(((k_hbm, kbuf, ksem), (v_hbm, vbuf, vsem))):
                pltpu.make_async_copy(
                    src.at[pl.ds(aligned(g * gd + row, 8), 8), pl.ds(seq - win + col, kv_cols)],
                    buf.at[slot, pl.ds(row, 8), pl.ds(col, kv_cols)],
                    sem.at[slot],
                ).start(priority=queue)
            return carry

        lax.fori_loop(0, kv_tiles // 2, issue, 0)

    def kv_wait(buf, sem, slot):
        pltpu.make_async_copy(buf.at[slot], buf.at[slot], sem.at[slot]).wait()

    def matrix_issue(src, dst, sem, piece_rows, piece_cols, streams):
        ncol = src.shape[1] // piece_cols
        col_bits = _log2(ncol)
        half = (src.shape[0] // piece_rows) * ncol // 2
        seg = half // streams

        def outer(j, carry):
            def inner(s, carry):
                for queue in range(2):
                    idx = queue * half + s * seg + j
                    r = pl.ds(aligned((idx >> col_bits) * piece_rows, 8), piece_rows)
                    c = pl.ds(aligned((idx & (ncol - 1)) * piece_cols, _LANE), piece_cols)
                    pltpu.make_async_copy(src.at[r, c], dst.at[r, c], sem).start(priority=queue)
                return carry

            return lax.fori_loop(0, streams, inner, carry)

        lax.fori_loop(0, seg, outer, 0)

    def full_wait(dst, sem):
        pltpu.make_async_copy(dst, dst, sem).wait()

    def wo_issue(first_pair, n_pairs):
        def issue(p, carry):
            j = p >> _log2(pairs_per_slice)
            i = p & (pairs_per_slice - 1)
            is_last = j == last
            s = jnp.where(is_last, i >> _log2(per_chunk), i & (seg_pairs - 1))
            t = jnp.where(is_last, i & (per_chunk - 1), i >> _log2(seg_pairs))
            sem_idx = jnp.where(is_last, last + (s >> _log2(seg_pairs // _WO_LAST_PARTS)), j)
            for queue in range(2):
                src_row = (s + queue * seg_pairs) * seg_rows + j * _WO_CHUNK + t * _WO_PIECE
                dst_row = (2 * s + queue) * _WO_CHUNK + t * _WO_PIECE
                pltpu.make_async_copy(
                    wo_hbm.at[pl.ds(aligned(src_row, 8), _WO_PIECE), :],
                    wo_v.at[j, pl.ds(aligned(dst_row, 8), _WO_PIECE), :],
                    wosem.at[sem_idx],
                ).start(priority=queue)
            return carry

        lax.fori_loop(first_pair, first_pair + n_pairs, issue, 0)

    small_copies = [
        pltpu.make_async_copy(src, dst, ssem.at[i])
        for i, (src, dst) in enumerate(((x_hbm, x_v), (gw_hbm, gw_v), (b1_hbm, b1_v), (b2_hbm, b2_v)))
    ]

    matrix_issue(wq_hbm, wq_v, wsem.at[0], 8, wq_v.shape[1] // 4, 5)
    for c in small_copies:
        c.start()
    matrix_issue(w1_hbm, w1_v, wsem.at[1], 8, d_ff, 5)
    matrix_issue(w2_hbm, w2_v, wsem.at[2], 24, d_model, 4)
    lax.fori_loop(0, steps, lambda t, carry: (kv_issue(0, 0, t), carry)[1], 0)

    for c in small_copies:
        c.wait()
    x = x_v[...]
    x_rows = jnp.broadcast_to(x, (_ROWS, d_model))
    gate = jax.nn.sigmoid(
        jnp.sum(x.astype(f32) * gw_v[...].astype(f32).reshape(1, d_model), axis=-1, keepdims=True))
    b1_f[...] = jnp.broadcast_to(b1_v[...].astype(f32).reshape(1, d_ff), (_ROWS, d_ff))
    full_wait(w1_v, wsem.at[1])
    full_wait(w2_v, wsem.at[2])

    def ffn_step(j, acc):
        @pl.when(j < steps)
        def _():
            kv_issue(1, 1, j)

        cs = pl.ds(aligned(j * _FF_CHUNK, _LANE), _FF_CHUNK)
        h = jnp.dot(x_rows, w1_v[:, cs], preferred_element_type=f32) + b1_f[:, cs]
        h = jax.nn.gelu(h.astype(bf16).astype(f32), approximate=True).astype(bf16)
        return acc + jnp.dot(h, w2_v[cs, :], preferred_element_type=f32)

    ffn = lax.fori_loop(0, d_ff // _FF_CHUNK, ffn_step, jnp.zeros((_ROWS, d_model), f32))
    ffn = ffn + b2_v[...].astype(f32).reshape(1, d_model)

    full_wait(wq_v, wsem.at[0])
    row = lax.broadcasted_iota(jnp.int32, (_ROWS, gd), 0)
    col = lax.broadcasted_iota(jnp.int32, (_ROWS, gd), 1)
    own = (col >= row * head_dim) & (col < (row + 1) * head_dim)

    wo_pairs_in_groups = (n_slices - 2) * pairs_per_slice
    wo_pairs_per_step = wo_pairs_in_groups // (_AHEAD * steps)

    def group_step(g, carry):
        slot = g % _NBUF
        next_slot = (g + _AHEAD) % _NBUF
        cols = pl.ds(aligned(g * gd, _LANE), gd)

        def issue(step):
            @pl.when(g + _AHEAD < n_groups)
            def _():
                kv_issue(g + _AHEAD, next_slot, step)

            @pl.when(g + _AHEAD >= n_groups)
            def _():
                wo_issue(((g + _AHEAD - n_groups) * steps + step) * wo_pairs_per_step, wo_pairs_per_step)

        q = jnp.dot(x_rows, wq_v[:, cols], preferred_element_type=f32)
        q_bd = jnp.where(own, q, 0.0).astype(bf16)

        kv_wait(kbuf, ksem, slot)

        def qk_step(c, m):
            issue(c)
            cs = pl.ds(aligned(c * kv_cols, _LANE), kv_cols)
            s = jnp.dot(q_bd, kbuf[slot, :, cs], preferred_element_type=f32) * (head_dim ** -0.5)
            s_scr[:, cs] = s
            return jnp.maximum(m, jnp.max(s, axis=-1, keepdims=True))

        m = lax.fori_loop(0, _KV_CHUNKS, qk_step, jnp.full((_ROWS, 1), -jnp.inf, f32))
        e = jnp.exp(s_scr[...] - m)
        p_scr[...] = (e / jnp.sum(e, axis=-1, keepdims=True)).astype(bf16)

        kv_wait(vbuf, vsem, slot)

        def pv_step(c, o):
            issue(_KV_CHUNKS + c)
            cs = pl.ds(aligned(c * kv_cols, _LANE), kv_cols)
            return o + lax.dot_general(p_scr[:, cs], vbuf[slot, :, cs], (((1,), (1,)), ((), ())),
                                       preferred_element_type=f32)

        o = lax.fori_loop(0, _KV_CHUNKS, pv_step, jnp.zeros((_ROWS, gd), f32))
        o_scr[:, cols] = jnp.where(own, o, 0.0).astype(bf16)
        return carry

    lax.fori_loop(0, n_groups, group_step, 0)

    def attn_cols(j, first_pair, n):
        return jnp.concatenate(
            [o_scr[:, pl.ds(aligned((first_pair + s + queue * seg_pairs) * seg_rows + j * _WO_CHUNK, _LANE),
                            _WO_CHUNK)]
             for s in range(n) for queue in range(2)], axis=1)

    def wo_step(j, acc):
        @pl.when(j < 2)
        def _():
            wo_issue(wo_pairs_in_groups + j * pairs_per_slice, pairs_per_slice)

        full_wait(wo_v.at[j], wosem.at[j])
        return acc + jnp.dot(attn_cols(j, 0, seg_pairs), wo_v[j], preferred_element_type=f32)

    acc = lax.fori_loop(0, last, wo_step, jnp.zeros((_ROWS, d_model), f32))

    part_pairs = seg_pairs // _WO_LAST_PARTS
    part_rows = 2 * part_pairs * _WO_CHUNK

    def wo_last_step(u, acc):
        rs = pl.ds(aligned(u * part_rows, 8), part_rows)
        full_wait(wo_v.at[last, rs], wosem.at[last + u])
        return acc + jnp.dot(attn_cols(last, u * part_pairs, part_pairs), wo_v[last, rs, :],
                             preferred_element_type=f32)

    acc = lax.fori_loop(0, _WO_LAST_PARTS, wo_last_step, acc)
    attn = jnp.sum(acc, axis=0, keepdims=True)
    o_ref[...] = (gate * attn + (1.0 - gate) * ffn[0:1]).astype(o_ref.dtype)


@jax.jit
def pallas_gated_mix__sliding_block_cached__dense_activation_gelu__decode_kernel(
    A_x: jax.Array,
    A_k_cache: jax.Array,
    A_v_cache: jax.Array,
    A_wq: jax.Array,
    A_wo: jax.Array,
    B_x: jax.Array,
    B_w1: jax.Array,
    B_b1: jax.Array,
    B_w2: jax.Array,
    B_b2: jax.Array,
    gate_w: jax.Array,
):
    del B_x
    batch, sq, d_model = A_x.shape
    _, n_heads, seq, head_dim = A_k_cache.shape
    d_ff = B_w1.shape[1]
    win = min(4096, max(256, seq // 4))
    gd = _HEADS_PER_GROUP * head_dim
    d_attn = n_heads * head_dim
    slice_rows = _WO_SEGS * _WO_CHUNK
    n_slices = d_attn // slice_rows
    assert batch * sq == 1 and A_wq.shape == (d_model, d_attn) and A_wo.shape == (d_attn, d_model)
    assert B_w1.shape == (d_model, d_ff) and B_w2.shape == (d_ff, d_model)
    assert n_heads % _HEADS_PER_GROUP == 0 and gd % _LANE == 0 and gd % 16 == 0
    assert n_heads // _HEADS_PER_GROUP > _AHEAD
    assert win % (_KV_CHUNKS * _LANE) == 0 and (seq - win) % _LANE == 0 and _KV_CHUNKS == 2
    assert d_ff % _FF_CHUNK == 0 and d_ff // _FF_CHUNK >= 2 * _KV_CHUNKS
    assert d_attn % slice_rows == 0 and n_slices > 2
    assert ((n_slices - 2) * (_WO_SEGS // 2) * (_WO_CHUNK // _WO_PIECE)) % (_AHEAD * 2 * _KV_CHUNKS) == 0
    assert d_attn % (4 * _LANE) == 0 and (d_model // 8 * 4) % (2 * 5) == 0
    assert d_model % 8 == 0 and (d_model // 8) % (2 * 5) == 0
    assert d_ff % 24 == 0 and (d_ff // 24) % (2 * 4) == 0

    k_t = jnp.swapaxes(A_k_cache, 2, 3).reshape(d_attn, seq)
    v_t = jnp.swapaxes(A_v_cache, 2, 3).reshape(d_attn, seq)

    bf16, f32 = jnp.bfloat16, jnp.float32
    hbm = pl.BlockSpec(memory_space=pl.ANY)
    out = pl.pallas_call(
        functools.partial(_kernel, head_dim=head_dim),
        in_specs=[hbm] * 10,
        out_specs=pl.BlockSpec(memory_space=pltpu.VMEM),
        out_shape=jax.ShapeDtypeStruct((1, d_model), A_x.dtype),
        scratch_shapes=[
            pltpu.VMEM((1, d_model), bf16),
            pltpu.VMEM((d_model,), bf16),
            pltpu.VMEM((d_ff,), bf16),
            pltpu.VMEM((d_model,), bf16),
            pltpu.VMEM((_NBUF, gd, win), bf16),
            pltpu.VMEM((_NBUF, gd, win), bf16),
            pltpu.VMEM(A_wq.shape, bf16),
            pltpu.VMEM((n_slices, slice_rows, d_model), bf16),
            pltpu.VMEM(B_w1.shape, bf16),
            pltpu.VMEM(B_w2.shape, bf16),
            pltpu.VMEM((_ROWS, d_attn), bf16),
            pltpu.VMEM((_ROWS, win), f32),
            pltpu.VMEM((_ROWS, win), bf16),
            pltpu.VMEM((_ROWS, d_ff), f32),
            pltpu.SemaphoreType.DMA((_NBUF,)),
            pltpu.SemaphoreType.DMA((_NBUF,)),
            pltpu.SemaphoreType.DMA((3,)),
            pltpu.SemaphoreType.DMA((4,)),
            pltpu.SemaphoreType.DMA((n_slices - 1 + _WO_LAST_PARTS,)),
        ],
        compiler_params=pltpu.CompilerParams(vmem_limit_bytes=64 * 1024 * 1024),
    )(A_x.reshape(1, d_model), gate_w, B_b1, B_b2, k_t, v_t, A_wq, A_wo, B_w1, B_w2)
    return out.reshape(batch, sq, d_model)
```
